```python
import jax
import jax.numpy as jnp

def _softmax(x, axis=-1):
    return jax.nn.softmax(x, axis=axis)

def _gelu(x):
    return jax.nn.gelu(x, approximate=True)

def _silu(x):
    return jax.nn.silu(x)

def _sigmoid(x):
    return jax.nn.sigmoid(x)

def _layernorm(x, axis=-1, eps=1e-05):
    m = jnp.mean(x, axis=axis, keepdims=True)
    v = jnp.var(x, axis=axis, keepdims=True)
    return (x - m) / jnp.sqrt(v + eps)

def _scatter_add(tgt, idx, src, axis=0):
    return tgt.at[idx].add(src)

def _segment_sum(src, seg, n):
    return jax.ops.segment_sum(src, seg, n)

class _Rng:

    def __init__(self, key):
        self._k = key

    def _next(self):
        self._k, sub = jax.random.split(self._k)
        return sub

    def normal(self, shape):
        return jax.random.normal(self._next(), shape, dtype=jnp.bfloat16)

    def randint(self, lo, hi, shape):
        return jax.random.randint(self._next(), shape, lo, hi, dtype=jnp.int32)

    def uniform(self, shape, lo=0.0, hi=1.0):
        return jax.random.uniform(self._next(), shape, jnp.bfloat16, lo, hi)

    def permutation(self, n):
        return jax.random.permutation(self._next(), n)
kernel_name = 'sequential_preLN__memory_aug_recurrent_mem_tr__mixer_s_mlp__prompt'

def setup_inputs():
    _rng = _Rng(jax.random.key(int.from_bytes(__import__("os").urandom(4), "little")))
    _w = lambda a: (lambda t: t.astype(jnp.bfloat16) if jnp.issubdtype(t.dtype, jnp.floating) else t)(jnp.asarray(a))

    def _A_setup():
        B, S, Dm = (1, 2048, 1024)
        H, Dh = (32, 128)
        M, seg = (8, 32)
        seg = min(seg, S)
        S = S // seg * seg
        return {'x': _w((lambda *s: _rng.normal(s) * 0.05)(B, S, Dm)), 'mem0': _w((lambda *s: _rng.normal(s) * 0.05)(B, M, Dm)), 'Wq': _w((lambda *s: _rng.normal(s) * 0.05)(Dm, H, Dh) * Dm ** (-0.5)), 'Wk': _w((lambda *s: _rng.normal(s) * 0.05)(Dm, H, Dh) * Dm ** (-0.5)), 'Wv': _w((lambda *s: _rng.normal(s) * 0.05)(Dm, H, Dh) * Dm ** (-0.5)), 'Wo': _w((lambda *s: _rng.normal(s) * 0.05)(H, Dh, Dm) * (H * Dh) ** (-0.5)), 'seg_len': seg}
    _A_in = _A_setup()

    def _B_setup():
        B, S, D, F = (1, 2048, 1024, 3584)
        return {'x': _w((lambda *s: _rng.normal(s) * 0.05)(B, S, D)), 'w1': _w((lambda *s: _rng.normal(s) * 0.05)(D, D) * D ** (-0.5)), 'w2': _w((lambda *s: _rng.normal(s) * 0.05)(D, D) * D ** (-0.5)), 'w3': _w((lambda *s: _rng.normal(s) * 0.05)(D, F) * D ** (-0.5)), 'w4': _w((lambda *s: _rng.normal(s) * 0.05)(F, D) * F ** (-0.5))}
    _B_in = _B_setup()
    return {'A_x': _A_in['x'], 'A_mem0': _A_in['mem0'], 'A_Wq': _A_in['Wq'], 'A_Wk': _A_in['Wk'], 'A_Wv': _A_in['Wv'], 'A_Wo': _A_in['Wo'], 'A_seg_len': _A_in['seg_len'], 'B_x': _B_in['x'], 'B_w1': _B_in['w1'], 'B_w2': _B_in['w2'], 'B_w3': _B_in['w3'], 'B_w4': _B_in['w4']}

def reference(A_x, A_mem0, A_Wq, A_Wk, A_Wv, A_Wo, A_seg_len, B_x, B_w1, B_w2, B_w3, B_w4):

    def _A_ref(x, mem0, Wq, Wk, Wv, Wo, seg_len):
        B, S, Dm = x.shape
        H, Dh = (Wq.shape[1], Wq.shape[2])
        M = mem0.shape[1]
        scale = Dh ** (-0.5)
        n_seg = S // seg_len
        L = M + seg_len
        idx = jnp.arange(L)
        mask = (idx[:, None] < M) | (idx[:, None] >= idx[None, :])
        mem = mem0
        outs = []
        for s in range(n_seg):
            xs = x[:, s * seg_len:(s + 1) * seg_len, :].copy()
            h = jnp.concatenate([mem, xs], axis=1)
            q = jnp.einsum('btd,dhe->bhte', h, Wq)
            k = jnp.einsum('btd,dhe->bhte', h, Wk)
            v = jnp.einsum('btd,dhe->bhte', h, Wv)
            scores = jnp.einsum('bhqe,bhke->bhqk', q, k) * scale
            scores = jnp.where(mask[None, None], scores, -1000000000.0)
            p = _softmax(scores, axis=-1)
            o = jnp.einsum('bhqk,bhke->bhqe', p, v)
            o = jnp.einsum('bhte,hed->btd', o, Wo)
            mem = o[:, :M, :].copy()
            outs.append(o[:, M:, :])
        return jnp.concatenate(outs, axis=1)

    def _B_ref(x, w1, w2, w3, w4):
        B, S, D = x.shape
        h = _gelu(_layernorm(x, axis=-1) @ w1)
        c = D // 4
        g0 = jnp.pad(h[:, :, 0 * c:1 * c], ((0, 0), (1, 0), (0, 0)))[:, :S, :]
        g1 = jnp.pad(h[:, :, 1 * c:2 * c], ((0, 0), (0, 1), (0, 0)))[:, 1:, :]
        g2 = jnp.pad(h[:, :, 2 * c:3 * c], ((0, 0), (2, 0), (0, 0)))[:, :S, :]
        g3 = jnp.pad(h[:, :, 3 * c:], ((0, 0), (0, 2), (0, 0)))[:, 2:, :]
        hs = jnp.concatenate([g0, g1, g2, g3], axis=-1) @ w2
        x1 = x + hs
        h2 = _gelu(_layernorm(x1, axis=-1) @ w3) @ w4
        return x1 + h2
    x = A_x
    h = x + _A_ref(_layernorm(x, axis=-1), A_mem0, A_Wq, A_Wk, A_Wv, A_Wo, A_seg_len)
    h2 = h + _B_ref(_layernorm(h, axis=-1), B_w1, B_w2, B_w3, B_w4)
    return h2
```

```python
import functools

import jax
import jax.numpy as jnp
import numpy as np
from jax import lax
from jax.experimental import pallas as pl
from jax.experimental.pallas import tpu as pltpu

bf16 = jnp.bfloat16
f32 = jnp.float32
u32 = jnp.uint32

S, D, H, E, F = 2048, 1024, 32, 128, 3584
M, SEG = 8, 32
L = M + SEG
NSEG = S // SEG
N = H * E
R0 = 512
CH = 24
RG = 544
HG = 8
NG = H // HG
EPS = 1e-5


def _dot(a, b):
  return lax.dot_general(a, b, (((1,), (0,)), ((), ())), preferred_element_type=f32)


def _dot_nt(a, b):
  return lax.dot_general(a, b, (((1,), (1,)), ((), ())), preferred_element_type=f32)


def _ln(x):
  m = jnp.mean(x, axis=-1, keepdims=True)
  xc = x - m
  v = jnp.mean(xc * xc, axis=-1, keepdims=True)
  return xc * lax.rsqrt(v + EPS)


def _gelu(x):
  return 0.5 * x * (1.0 + jnp.tanh(0.7978845608028654 * (x + 0.044715 * (x * x * x))))


ORDERS = {
    'J': "q0 k0 v0 qk0 q1 k1 v1 pv0 qk1 q2 k2 v2 pv1 qk2 q3 k3 v3 pv2 qk3 wo0-1 wo2-2 pv3 wo3-3",
    'L': "q0 k0 v0 qk0 q1 k1 v1 pv0 qk1 q2 k2 v2 pv1 qk2 q3 k3 v3 pv2 wo0-0 qk3 wo1-2 pv3 wo3-3",
    'F': "q0 k0 v0 qk0 q1 k1 pv0 v1 qk1 q2 k2 pv1 v2 qk2 q3 k3 pv2 qk3 v3 wo0-1 wo2-2 pv3 wo3-3",
}


def _parse(s):
  out = []
  for t in s.split():
    if t.startswith('wo'):
      a, b = t[2:].split('-')
      out.append(('wo', int(a) * HG, (int(b) + 1) * HG))
    elif t.startswith('qk'):
      out.append(('qk', int(t[2:])))
    elif t.startswith('pv'):
      out.append(('pv', int(t[2:])))
    else:
      out.append((t[0], int(t[1:])))
  return out


def make_kernel(order='J', RB=256, phases="PAB", unroll=2, bvar='halves2', tag='', ramp=True, WSL=8, tdist=1):
  scale = E ** -0.5
  NB = S // RB
  ops = _parse(ORDERS.get(order, order))
  NU = 3 * NG

  def kernel(x_hbm, mem0_hbm, wq_hbm, wk_hbm, wv_hbm, wo_hbm, w1_hbm, w2_hbm, w3_hbm, w4_hbm,
             out_hbm, *scr):
    (x_v, mem_v, xln_v, zero_v), scr = scr[:4], scr[4:]
    wpk, scr = scr[:NU], scr[NU:]
    ring, scr = scr[:NU], scr[NU:]
    (wo_pk, h_v, g_v, w1_v, w2_v, w3_v, w4_v, out_v,
     sem_x, sem_u, sem_w, sem_out) = scr
    whbm = [r.bitcast(u32) for r in (wq_hbm, wk_hbm, wv_hbm)]

    def unit_cps(u):
      m, g = divmod(u, NG)
      cps = []
      for par in range(2):
        for hpl in range(HG // 2):
          cps.append(pltpu.make_async_copy(
              whbm[m].at[:, par * (H // 2) + g * (HG // 2) + hpl, :],
              wpk[u].at[par * (HG // 2) + hpl], sem_u.at[u]))
      return cps

    x_cp0 = pltpu.make_async_copy(x_hbm.at[pl.ds(0, R0)], x_v.at[pl.ds(0, R0)], sem_x.at[0])
    x_cp1 = pltpu.make_async_copy(x_hbm.at[pl.ds(R0, S - R0)], x_v.at[pl.ds(R0, S - R0)], sem_x.at[1])
    mem_cp = pltpu.make_async_copy(mem0_hbm, mem_v, sem_x.at[2])
    NWO = 4
    wo_cps = [pltpu.make_async_copy(wo_hbm.bitcast(u32).at[pl.ds(i * (N // 2 // NWO), N // 2 // NWO)],
                                    wo_pk.at[pl.ds(i * (N // 2 // NWO), N // 2 // NWO)], sem_w.at[i])
              for i in range(NWO)]
    b_cps = [pltpu.make_async_copy(a, b, sem_w.at[NWO + i]) for i, (a, b) in enumerate(
        ((w1_hbm, w1_v), (w2_hbm, w2_v), (w3_hbm, w3_v), (w4_hbm, w4_v)))]

    nsub = NU + 2 if ramp else NU
    off = 2 if ramp else 0
    XW = off + 3
    extra = {off + 1: [x_cp1]}
    for j, c in enumerate(wo_cps):
      extra.setdefault(off + 3 + j, []).append(c)
    if "B" in phases:
      for j, c in enumerate(b_cps):
        extra.setdefault(off + 7 + j, []).append(c)
    lnplan = {}
    groups = list(range(R0, S, 16))
    slots = [(i, sl) for i in range(XW, nsub) for sl in range(16)]
    for j, r in enumerate(groups):
      lnplan.setdefault(slots[(j * len(slots)) // len(groups)], []).append(r)

    def fix_vals(ref, hpl, rows):
      a = ref[hpl, rows, :]
      c = ref[HG // 2 + hpl, rows, :]
      lo = (a & jnp.uint32(0xFFFF)) | (c << 16)
      hi = (a >> 16) | (c & jnp.uint32(0xFFFF0000))
      ref[hpl, rows, :] = lo
      ref[HG // 2 + hpl, rows, :] = hi
      return lo | hi

    def rhs(u):
      return pltpu.bitcast(jnp.concatenate(
          [wpk[u][(hl % 2) * (HG // 2) + hl // 2] for hl in range(HG)], axis=1), bf16)

    def ln_rows(r, n):
      y = _ln(x_v[pl.ds(r, n), :].astype(f32)).astype(bf16)
      xln_v[pl.ds(r, n), :] = y
      return y

    HP = HG // 2
    subs = [(0, 0, 1), (0, 1, 2), (0, 2, 4)] + [(u, 0, HP) for u in range(1, NU)] if ramp else [(u, 0, HP) for u in range(NU)]
    NSUB = len(subs)

    def sub_cps(i):
      u, a, b = subs[i]
      m, g = divmod(u, NG)
      return [pltpu.make_async_copy(
          whbm[m].at[:, par * (H // 2) + g * HP + hpl, :], wpk[u].at[par * HP + hpl], sem_u.at[i])
          for hpl in range(a, b) for par in range(2)]

    def start_all(cs):
      for c in cs:
        c.start()

    def wait_all(cs):
      for c in cs:
        c.wait()

    def fix_chunk(i, r0, nrows):
      u, a, b = subs[i]
      acc = None
      for hpl in range(a, b):
        t = fix_vals(wpk[u], hpl, pl.ds(r0, nrows))
        for q in range(nrows // 8):
          acc = t[8 * q:8 * q + 8] if acc is None else acc | t[8 * q:8 * q + 8]
      return acc

    def tie(lhs, dep):
      lu = pltpu.bitcast(lhs[0:16, 0:E], u32) | dep
      return jnp.concatenate(
          [jnp.concatenate([pltpu.bitcast(lu, bf16), lhs[0:16, E:]], axis=1), lhs[16:, :]], axis=0)

    x_cp0.start()
    start_all(sub_cps(0))
    mem_cp.start()
    zero_v[...] = jnp.zeros(zero_v.shape, u32)
    with jax.named_scope("xwait"):
      x_cp0.wait()
      wait_all(sub_cps(0))
    start_all(sub_cps(1))
    start_all(sub_cps(2))
    with jax.named_scope("fix0"):
      for b in range(8):
        fix_chunk(0, b * 64, 64)

    NSL = 16
    RS = R0 // NSL
    zero = zero_v[...]
    for i, (u, a, b) in enumerate(subs):
      with jax.named_scope(f"unit{i:02d}"):
        c0, c1 = 2 * a * E, 2 * b * E
        deps = {}
        if i == 0:
          ln_rows(0, RS)
        for sl in range(NSL):
          if sl == WSL and i + 1 < NSUB:
            wait_all(sub_cps(i + 1))
            if i + 3 < NSUB:
              start_all(sub_cps(i + 3))
            for c in extra.get(i, ()):
              c.start()
          if sl == 0 and i == XW:
            x_cp1.wait()
          w = pltpu.bitcast(jnp.concatenate(
              [wpk[u][(hl % 2) * HP + hl // 2] for hl in range(2 * a, 2 * b)], axis=1), bf16)
          lhs = xln_v[pl.ds(sl * RS, RS), :]
          if sl in deps:
            lhs = tie(lhs, deps.pop(sl) & zero)
          ring[u][pl.ds(sl * RS, RS), c0:c1] = _dot(lhs, w)

          def add_dep(t, at):
            at = min(at, NSL - 1)
            if at > sl:
              deps[at] = t if at not in deps else deps[at] | t
          if i == 0 and sl + 1 < NSL:
            ln_rows((sl + 1) * RS, RS)
          if i + 1 < NSUB and sl >= WSL:
            nfs = NSL - 1 - WSL
            k = sl - WSL
            if k < nfs:
              lo, hi = (k * 64) // nfs * 8, ((k + 1) * 64) // nfs * 8
              if hi > lo:
                add_dep(fix_chunk(i + 1, lo, hi - lo), sl + tdist)
          for r in lnplan.get((i, sl), ()):
            y = ln_rows(r, 16)
            add_dep(pltpu.bitcast(y[:, 0:E], u32), sl + tdist)

    for c in wo_cps:
      c.wait()
    mem_cp.wait()

    ri = lax.broadcasted_iota(jnp.int32, (L, L), 0)
    ci = lax.broadcasted_iota(jnp.int32, (L, L), 1)
    mask = (ri < M) | (ri >= ci)

    def step(s, carry):
      mem, wp, rpos = carry
      rc = pl.multiple_of(R0 + CH * s, 8)
      lhs = jnp.concatenate([xln_v[pl.ds(rc, CH), :], mem.astype(bf16)], axis=0)
      wpos = [pl.multiple_of(wp, 8)]
      for i in range(CH // 8):
        t = wpos[-1] + 8
        wpos.append(pl.multiple_of(jnp.where(t >= RG, t - RG, t), 8))
      rpos = pl.multiple_of(rpos, SEG)
      rnext = jnp.where(rpos + SEG >= RG, 0, rpos + SEG)
      val = {}
      os_ = {}
      st = dict(acc=None)

      def proj(m, g):
        u = m * NG + g
        y = _dot(lhs, rhs(u))
        for i in range(CH // 8):
          ring[u][pl.ds(wpos[i], 8), :] = y[8 * i:8 * (i + 1), :]
        val[(m, g)] = y[CH:, :]

      def full(m, g):
        tok = ring[m * NG + g][pl.ds(rpos, SEG), :]
        return jnp.concatenate([val[(m, g)], tok], axis=0)

      def qk(g):
        q = full(0, g)
        k = full(1, g)
        for hh in range(HG):
          sl = slice(hh * E, (hh + 1) * E)
          sc = _dot_nt(q[:, sl], k[:, sl]) * scale
          sc = jnp.where(mask, sc, -1e9)
          mx = jnp.max(sc, axis=-1, keepdims=True)
          e = jnp.exp(sc - mx)
          l = jnp.sum(e, axis=-1, keepdims=True)
          r = pl.reciprocal(l, approx=True)
          r = r * (2.0 - l * r)
          val[('p', g * HG + hh)] = (e, r)

      def pv(g):
        v = full(2, g)
        for hh in range(HG):
          sl = slice(hh * E, (hh + 1) * E)
          e, r = val[('p', g * HG + hh)]
          os_[g * HG + hh] = _dot(e, v[:, sl]) * r

      def wo(h0, h1):
        o = jnp.concatenate([os_[h] for h in range(h0, h1)], axis=1)
        part = _dot(o, pltpu.bitcast(wo_pk[h0 * E // 2:h1 * E // 2, :], bf16))
        st['acc'] = part if st['acc'] is None else st['acc'] + part

      for op in ops:
        if op[0] == 'qk':
          qk(op[1])
        elif op[0] == 'pv':
          pv(op[1])
        elif op[0] == 'wo':
          wo(op[1], op[2])
        else:
          proj('qkv'.index(op[0]), op[1])
      acc = st['acc']
      r0 = pl.multiple_of(s * SEG, SEG)
      h_v[pl.ds(r0, SEG), :] = acc[M:, :] + x_v[pl.ds(r0, SEG), :].astype(f32)
      return acc[:M, :], wpos[CH // 8], rnext

    if "A" in phases:
      with jax.named_scope("steps"):
        lax.fori_loop(0, NSEG, step, (mem_v[...].astype(f32), jnp.int32(R0), jnp.int32(0)), unroll=unroll)
    else:
      for u in range(NU):
        h_v[pl.ds(0, RB), :] = x_v[pl.ds(0, RB), :].astype(f32) + ring[u][pl.ds(0, RB), :]

    def out_cp(b, slot):
      return pltpu.make_async_copy(out_v.at[slot], out_hbm.at[pl.ds(b * RB, RB)], sem_out.at[slot])

    if "B" in phases:
      for c in b_cps:
        c.wait()
      zero8 = jnp.zeros((8, D), f32)
      g_v[pl.ds(0, 8), :] = zero8
      g_v[pl.ds(S + 8, 8), :] = zero8
      c4 = D // 4

      def al(r):
        return r if isinstance(r, int) else pl.multiple_of(r, 8)

      def w1job(r0, n):
        z = _ln(_ln(h_v[pl.ds(al(r0), n), :])).astype(bf16)
        g_v[pl.ds(al(r0 + 8), n), :] = _gelu(_dot(z, w1_v[...]))

      def shifted(r0, n):
        gw = g_v[pl.ds(al(r0), n + 16), :]
        return jnp.concatenate([gw[7:7 + n, 0:c4], gw[9:9 + n, c4:2 * c4],
                                gw[6:6 + n, 2 * c4:3 * c4], gw[10:10 + n, 3 * c4:]], axis=1).astype(bf16)

      def bbody(b, last):
        r = b * RB
        n = RB // 2
        slot = b % 2
        if not last:
          @pl.when(b >= 2)
          def _():
            out_cp(b - 2, slot).wait()
        else:
          out_cp(b - 2, slot).wait()
        hA = h_v[pl.ds(al(r), n), :]
        hB = h_v[pl.ds(al(r + n), n), :]
        x1A = _ln(hA) + _dot(shifted(r, n), w2_v[...])
        if not last:
          w1job(r + RB, n)
        tA = _gelu(_dot(_ln(x1A).astype(bf16), w3_v[...])).astype(bf16)
        x1B = _ln(hB) + _dot(shifted(r + n, n), w2_v[...])
        if not last:
          w1job(r + RB + n, n)
        oA = _dot(tA, w4_v[...])
        tB = _gelu(_dot(_ln(x1B).astype(bf16), w3_v[...])).astype(bf16)
        out_v[slot, pl.ds(0, n), :] = (hA + x1A + oA).astype(bf16)
        out_v[slot, pl.ds(n, n), :] = (hB + x1B + _dot(tB, w4_v[...])).astype(bf16)
        out_cp(b, slot).start()

      with jax.named_scope("b1first"):
        w1job(0, RB // 2)
        w1job(RB // 2, RB // 2)

      with jax.named_scope("bloop"):
        lax.fori_loop(0, NB - 1, lambda b, _: bbody(b, False), None)
      with jax.named_scope("blast"):
        bbody(NB - 1, True)
        out_cp(NB - 2, (NB - 2) % 2).wait()
        out_cp(NB - 1, (NB - 1) % 2).wait()
    else:
      out_v[0] = h_v[pl.ds(0, RB), :].astype(bf16)
      out_cp(0, 0).start()
      out_cp(0, 0).wait()

  scratch = [
      pltpu.VMEM((S, D), bf16),
      pltpu.VMEM((M, D), bf16),
      pltpu.VMEM((S, D), bf16),
      pltpu.VMEM((8, E), u32),
  ] + [pltpu.VMEM((HG, D // 2, E), u32)] * NU + [pltpu.VMEM((RG, HG * E), f32)] * NU + [
      pltpu.VMEM((N // 2, D), u32),
      pltpu.VMEM((S, D), f32),
      pltpu.VMEM((S + 16, D), f32),
      pltpu.VMEM((D, D), bf16), pltpu.VMEM((D, D), bf16),
      pltpu.VMEM((D, F), bf16), pltpu.VMEM((F, D), bf16),
      pltpu.VMEM((2, RB, D), bf16),
      pltpu.SemaphoreType.DMA((3,)),
      pltpu.SemaphoreType.DMA((NU + 2,)),
      pltpu.SemaphoreType.DMA((8,)),
      pltpu.SemaphoreType.DMA((2,)),
  ]

  def fn(A_x, A_mem0, A_Wq, A_Wk, A_Wv, A_Wo, A_seg_len, B_x, B_w1, B_w2, B_w3, B_w4):
    del A_seg_len, B_x
    out = pl.pallas_call(
        kernel,
        in_specs=[pl.BlockSpec(memory_space=pl.ANY)] * 10,
        out_specs=pl.BlockSpec(memory_space=pl.ANY),
        out_shape=jax.ShapeDtypeStruct((S, D), bf16),
        scratch_shapes=scratch,
        compiler_params=pltpu.CompilerParams(vmem_limit_bytes=124 * 2**20),
        name=f"k2_{RB}_{phases}_{unroll}_{tag}",
    )(A_x.reshape(S, D), A_mem0.reshape(M, D),
      A_Wq.reshape(D // 2, 2 * H, E), A_Wk.reshape(D // 2, 2 * H, E), A_Wv.reshape(D // 2, 2 * H, E),
      A_Wo.reshape(N, D), B_w1, B_w2, B_w3, B_w4)
    return out.reshape(1, S, D)
  return fn


_KERNEL_FN = make_kernel()


@functools.partial(jax.jit, static_argnames=("A_seg_len",))
def pallas_sequential_preLN__memory_aug_recurrent_mem_tr__mixer_s_mlp__prompt_kernel(
    A_x, A_mem0, A_Wq, A_Wk, A_Wv, A_Wo, A_seg_len, B_x, B_w1, B_w2, B_w3, B_w4):
  assert int(A_seg_len) == SEG, "kernel is built for the reference's fixed segment length"
  assert A_x.shape == (1, S, D) and A_mem0.shape == (1, M, D) and A_Wq.shape == (D, H, E)
  assert B_w3.shape == (D, F)
  return _KERNEL_FN(A_x, A_mem0, A_Wq, A_Wk, A_Wv, A_Wo, A_seg_len, B_x, B_w1, B_w2, B_w3, B_w4)
```

```python
import functools

import jax
import jax.numpy as jnp
import numpy as np
from jax import lax
from jax.experimental import pallas as pl
from jax.experimental.pallas import tpu as pltpu

bf16 = jnp.bfloat16
f32 = jnp.float32
u32 = jnp.uint32

S, D, H, E, F = 2048, 1024, 32, 128, 3584
M, SEG = 8, 32
L = M + SEG
NSEG = S // SEG
N = H * E
R0 = 512
CH = 24
RG = 544
HG = 8
NG = H // HG
EPS = 1e-5


def _dot(a, b):
  return lax.dot_general(a, b, (((1,), (0,)), ((), ())), preferred_element_type=f32)


def _dot_nt(a, b):
  return lax.dot_general(a, b, (((1,), (1,)), ((), ())), preferred_element_type=f32)


def _ln(x):
  m = jnp.mean(x, axis=-1, keepdims=True)
  xc = x - m
  v = jnp.mean(xc * xc, axis=-1, keepdims=True)
  return xc * lax.rsqrt(v + EPS)


def _gelu(x):
  return 0.5 * x * (1.0 + jnp.tanh(0.7978845608028654 * (x + 0.044715 * (x * x * x))))


ORDERS = {
    'J': "q0 k0 v0 qk0 q1 k1 v1 pv0 qk1 q2 k2 v2 pv1 qk2 q3 k3 v3 pv2 qk3 wo0-1 wo2-2 pv3 wo3-3",
    'L': "q0 k0 v0 qk0 q1 k1 v1 pv0 qk1 q2 k2 v2 pv1 qk2 q3 k3 v3 pv2 wo0-0 qk3 wo1-2 pv3 wo3-3",
    'F': "q0 k0 v0 qk0 q1 k1 pv0 v1 qk1 q2 k2 pv1 v2 qk2 q3 k3 pv2 qk3 v3 wo0-1 wo2-2 pv3 wo3-3",
}


def _parse(s):
  out = []
  for t in s.split():
    if t.startswith('wo'):
      a, b = t[2:].split('-')
      out.append(('wo', int(a) * HG, (int(b) + 1) * HG))
    elif t.startswith('qk'):
      out.append(('qk', int(t[2:])))
    elif t.startswith('pv'):
      out.append(('pv', int(t[2:])))
    else:
      out.append((t[0], int(t[1:])))
  return out


def make_kernel(order='J', RB=128, phases="PAB", unroll=2, bvar='halves2', tag='', ramp=((0, 0, 1), (0, 1, 2), (0, 2, 4), (1, 0, 2), (1, 2, 4)), nself=3, WSL=4, tdist=1, NSL=8, lnrows=16, pdma=False, usetie=True, noP=False, nodep=False, memfirst=False, noh=False, lnA=True, lnpos=('q', 1), lntie=('q', 2), WSL2={2: 6}, PD0=5, PDEP=3, x1at=8):
  scale = E ** -0.5
  NB = S // RB
  ops = _parse(ORDERS.get(order, order))
  NU = 3 * NG

  def kernel(z_smem, x_hbm, mem0_hbm, wq_hbm, wk_hbm, wv_hbm, wo_hbm, w1_hbm, w2_hbm, w3_hbm, w4_hbm,
             out_hbm, *scr):
    (x_v, mem_v, xln_v, zero_v), scr = scr[:4], scr[4:]
    wpk, scr = scr[:NU], scr[NU:]
    ring, scr = scr[:NU], scr[NU:]
    (wo_pk, h_v, g_v, w1_v, w2_v, w3_v, w4_v, out_v,
     sem_x, sem_u, sem_w, sem_out) = scr
    whbm = [r.bitcast(u32) for r in (wq_hbm, wk_hbm, wv_hbm)]

    def unit_cps(u):
      m, g = divmod(u, NG)
      cps = []
      for par in range(2):
        for hpl in range(HG // 2):
          cps.append(pltpu.make_async_copy(
              whbm[m].at[:, par * (H // 2) + g * (HG // 2) + hpl, :],
              wpk[u].at[par * (HG // 2) + hpl], sem_u.at[u]))
      return cps

    x_cp1 = pltpu.make_async_copy(x_hbm.at[pl.ds(R0, S - R0)], x_v.at[pl.ds(R0, S - R0)], sem_x.at[4])
    mem_cp = pltpu.make_async_copy(mem0_hbm, mem_v, sem_x.at[5])
    NWO = 4
    wo_cps = [pltpu.make_async_copy(wo_hbm.bitcast(u32).at[pl.ds(i * (N // 2 // NWO), N // 2 // NWO)],
                                    wo_pk.at[pl.ds(i * (N // 2 // NWO), N // 2 // NWO)], sem_w.at[i])
              for i in range(NWO)]
    b_cps = [pltpu.make_async_copy(a.bitcast(u32), b, sem_w.at[NWO + i]) for i, (a, b) in enumerate(
        ((w1_hbm, w1_v), (w2_hbm, w2_v), (w3_hbm, w3_v), (w4_hbm, w4_v)))]

    off = len(ramp) - ramp[-1][0] - 1
    nsub = NU + off
    XW = nsub - 1 if lnA else off + 3
    extra = {(x1at if x1at is not None else off + 1): [x_cp1]}
    for j, c in enumerate(wo_cps):
      extra.setdefault(off + 3 + j, []).append(c)
    if "B" in phases or pdma:
      for j, c in enumerate(b_cps):
        extra.setdefault(off + 7 + j, []).append(c)
    lnplan = {}
    groups = list(range(R0, R0 + 32, lnrows)) if lnA else list(range(R0, S, lnrows))
    slots = [(i, sl) for i in range(XW, nsub) for sl in range(NSL - 1)]
    for j, r in enumerate(groups):
      lnplan.setdefault(slots[(j * len(slots)) // len(groups)], []).append(r)

    def fix_vals(ref, hpl, rows):
      a = ref[hpl, rows, :]
      c = ref[HG // 2 + hpl, rows, :]
      lo = (a & jnp.uint32(0xFFFF)) | (c << 16)
      hi = (a >> 16) | (c & jnp.uint32(0xFFFF0000))
      ref[hpl, rows, :] = lo
      ref[HG // 2 + hpl, rows, :] = hi
      return lo | hi

    def rhs(u):
      return pltpu.bitcast(jnp.concatenate(
          [wpk[u][(hl % 2) * (HG // 2) + hl // 2] for hl in range(HG)], axis=1), bf16)

    def ln_rows(r, n):
      y = _ln(x_v[pl.ds(r, n), :].astype(f32)).astype(bf16)
      xln_v[pl.ds(r, n), :] = y
      return y

    HP = HG // 2
    subs = list(ramp) + [(u, 0, HP) for u in range(ramp[-1][0] + 1, NU)]
    NSUB = len(subs)

    def sub_cps(i):
      u, a, b = subs[i]
      m, g = divmod(u, NG)
      return [pltpu.make_async_copy(
          whbm[m].at[:, par * (H // 2) + g * HP + hpl, :], wpk[u].at[par * HP + hpl], sem_u.at[i])
          for hpl in range(a, b) for par in range(2)]

    def start_all(cs):
      for c in cs:
        c.start()

    def wait_all(cs):
      for c in cs:
        c.wait()

    def fix_chunk(i, r0, nrows):
      u, a, b = subs[i]
      acc = None
      for hpl in range(a, b):
        t = fix_vals(wpk[u], hpl, pl.ds(r0, nrows))
        for q in range(nrows // 8):
          acc = t[8 * q:8 * q + 8] if acc is None else acc | t[8 * q:8 * q + 8]
      return acc

    def tie(lhs, dep):
      lu = pltpu.bitcast(lhs[0:16, 0:E], u32) | dep
      return jnp.concatenate(
          [jnp.concatenate([pltpu.bitcast(lu, bf16), lhs[0:16, E:]], axis=1), lhs[16:, :]], axis=0)

    zero = jnp.full((8, E), z_smem[0], jnp.int32).astype(u32)
    one = z_smem[0] + 1
    HU = whbm[0]
    NXC = 4
    XC = R0 // NXC

    def xc_cp(c):
      return pltpu.make_async_copy(x_hbm.at[pl.ds(c * XC, XC)], x_v.at[pl.ds(c * XC, XC)], sem_x.at[c])

    def in_block(fn, n=1):
      lax.fori_loop(0, one * n, lambda i, _: fn(i), None)

    def start_sub_dyn(i):
      u, a, b = subs[i]
      m, g = divmod(u, NG)

      def body(j):
        hpl = a + j // 2
        par = j % 2
        pltpu.make_async_copy(whbm[m].at[:, par * (H // 2) + g * HP + hpl, :],
                              wpk[u].at[par * HP + hpl], sem_u.at[i]).start()
      in_block(body, 2 * (b - a))

    in_block(lambda i: xc_cp(0).start())
    start_sub_dyn(0)
    in_block(lambda i: pltpu.make_async_copy(
        x_hbm.at[pl.ds(pl.multiple_of((i + 1) * XC, XC), XC)],
        x_v.at[pl.ds(pl.multiple_of((i + 1) * XC, XC), XC)], sem_x.at[i + 1]).start(), NXC - 1)
    for i in range(1, PD0):
      start_sub_dyn(i)
    mem_cp.start()

    started = [PD0]
    RS = R0 // NSL
    SPC = XC // RS

    def fix_all(i):
      for bb in range(8):
        fix_chunk(i, bb * 64, 64)

    for i, (u, a, b) in enumerate(subs):
      with jax.named_scope(f"unit{i:02d}"):
        c0, c1 = 2 * a * E, 2 * b * E
        deps = {}
        if i == 0:
          xc_cp(0).wait()
          ln_rows(0, XC)
          wait_all(sub_cps(0))
          fix_all(0)
        elif i < nself:
          wait_all(sub_cps(i))
          fix_all(i)
        for sl in range(NSL):
          if i == 0 and sl % SPC == 0 and sl // SPC + 1 < NXC:
            xc_cp(sl // SPC + 1).wait()
          if sl == WSL2.get(i, WSL) and i + 1 < NSUB:
            if i + 1 >= nself:
              wait_all(sub_cps(i + 1))
            for j in range(started[0], min(i + PDEP + 1, NSUB)):
              start_all(sub_cps(j))
            started[0] = max(started[0], min(i + PDEP + 1, NSUB))
            for c in extra.get(i, ()):
              c.start()
          if sl == 0 and i == XW:
            x_cp1.wait()
          if noP:
            continue
          w = pltpu.bitcast(jnp.concatenate(
              [wpk[u][(hl % 2) * HP + hl // 2] for hl in range(2 * a, 2 * b)], axis=1), bf16)
          lhs = xln_v[pl.ds(sl * RS, RS), :]
          if sl in deps and usetie:
            lhs = tie(lhs, deps.pop(sl) & zero)
          ring[u][pl.ds(sl * RS, RS), c0:c1] = _dot(lhs, w)

          def add_dep(t, at):
            at = min(at, NSL - 1)
            if at > sl:
              deps[at] = t if at not in deps else deps[at] | t
          if i == 0 and sl % SPC == 0 and sl // SPC + 1 < NXC:
            ln_rows((sl // SPC + 1) * XC, XC)
          if nself <= i + 1 < NSUB and sl >= WSL2.get(i, WSL):
            ws = WSL2.get(i, WSL)
            nfs = max(NSL - 1 - ws, 1)
            k = sl - ws
            if k < nfs:
              lo, hi = (k * 64) // nfs * 8, ((k + 1) * 64) // nfs * 8
              if hi > lo:
                add_dep(fix_chunk(i + 1, lo, hi - lo), sl + tdist)
          for r in lnplan.get((i, sl), ()):
            y = ln_rows(r, lnrows)
            t = pltpu.bitcast(y[0:16, 0:E], u32)
            for q in range(1, lnrows // 16):
              t = t | pltpu.bitcast(y[16 * q:16 * q + 16, 0:E], u32)
            add_dep(t, sl + tdist)

    for c in wo_cps:
      c.wait()
    mem_cp.wait()

    ri = lax.broadcasted_iota(jnp.int32, (L, L), 0)
    ci = lax.broadcasted_iota(jnp.int32, (L, L), 1)
    mask = (ri < M) | (ri >= ci)

    def step(s, carry):
      mem, wp, rpos = carry
      rc = pl.multiple_of(R0 + CH * s, 8)
      mem_in = mem
      if nodep:
        mem = mem_v[...].astype(f32)
      if memfirst:
        lhs = jnp.concatenate([mem.astype(bf16), xln_v[pl.ds(rc, CH), :]], axis=0)
      else:
        lhs = jnp.concatenate([xln_v[pl.ds(rc, CH), :], mem.astype(bf16)], axis=0)
      lnst = dict(dep=None, used=False)
      t0 = M if memfirst else 0
      m0 = 0 if memfirst else CH
      wpos = [pl.multiple_of(wp, 8)]
      for i in range(CH // 8):
        t = wpos[-1] + 8
        wpos.append(pl.multiple_of(jnp.where(t >= RG, t - RG, t), 8))
      rpos = pl.multiple_of(rpos, SEG)
      rnext = jnp.where(rpos + SEG >= RG, 0, rpos + SEG)
      val = {}
      os_ = {}
      st = dict(acc=None)

      def proj(m, g):
        u = m * NG + g
        lh = lhs
        if lnA and ('qkv'[m], g) == lntie:
          lh = tie(lhs, lnst['dep'] & zero)
        y = _dot(lh, rhs(u))
        if lnA and ('qkv'[m], g) == lnpos:
          rn = pl.multiple_of(jnp.minimum(rc + CH, S - CH), 8)
          yl = _ln(x_v[pl.ds(rn, CH), :].astype(f32)).astype(bf16)
          xln_v[pl.ds(rn, CH), :] = yl
          d = None
          for q in range(D // E):
            t = pltpu.bitcast(yl[0:16, q * E:(q + 1) * E], u32)
            d = t if d is None else d | t
          lnst['dep'] = d
        for i in range(CH // 8):
          ring[u][pl.ds(wpos[i], 8), :] = y[t0 + 8 * i:t0 + 8 * (i + 1), :]
        val[(m, g)] = y[m0:m0 + M, :]

      def full(m, g):
        tok = ring[m * NG + g][pl.ds(rpos, SEG), :]
        return jnp.concatenate([val[(m, g)], tok], axis=0)

      def qk(g):
        q = full(0, g)
        k = full(1, g)
        for hh in range(HG):
          sl = slice(hh * E, (hh + 1) * E)
          sc = _dot_nt(q[:, sl], k[:, sl]) * scale
          sc = jnp.where(mask, sc, -1e9)
          mx = jnp.max(sc, axis=-1, keepdims=True)
          e = jnp.exp(sc - mx)
          l = jnp.sum(e, axis=-1, keepdims=True)
          r = pl.reciprocal(l, approx=True)
          r = r * (2.0 - l * r)
          val[('p', g * HG + hh)] = (e, r)

      def pv(g):
        v = full(2, g)
        for hh in range(HG):
          sl = slice(hh * E, (hh + 1) * E)
          e, r = val[('p', g * HG + hh)]
          os_[g * HG + hh] = _dot(e, v[:, sl]) * r

      def wo(h0, h1):
        o = jnp.concatenate([os_[h] for h in range(h0, h1)], axis=1)
        part = _dot(o, pltpu.bitcast(wo_pk[h0 * E // 2:h1 * E // 2, :], bf16))
        st['acc'] = part if st['acc'] is None else st['acc'] + part

      for op in ops:
        if op[0] == 'qk':
          qk(op[1])
        elif op[0] == 'pv':
          pv(op[1])
        elif op[0] == 'wo':
          wo(op[1], op[2])
        else:
          proj('qkv'.index(op[0]), op[1])
      acc = st['acc']
      r0 = pl.multiple_of(s * SEG, SEG)
      if noh:
        h_v[pl.ds(r0, SEG), :] = acc[M:, :]
      else:
        h_v[pl.ds(r0, SEG), :] = acc[M:, :] + x_v[pl.ds(r0, SEG), :].astype(f32)
      return acc[:M, :], wpos[CH // 8], rnext

    if "A" in phases:
      with jax.named_scope("steps"):
        lax.fori_loop(0, NSEG, step, (mem_v[...].astype(f32), jnp.int32(R0), jnp.int32(0)), unroll=unroll)
    else:
      for u in range(NU):
        h_v[pl.ds(0, RB), :] = x_v[pl.ds(0, RB), :].astype(f32) + ring[u][pl.ds(0, RB), :]

    def out_cp(b, slot):
      return pltpu.make_async_copy(out_v.at[slot], out_hbm.at[pl.ds(b * RB, RB)], sem_out.at[slot])

    if "B" in phases:
      for c in b_cps:
        c.wait()
      zero8 = jnp.zeros((8, D), f32)
      g_v[pl.ds(0, 8), :] = zero8
      g_v[pl.ds(S + 8, 8), :] = zero8
      c4 = D // 4
      W = lambda r: pltpu.bitcast(r[...], bf16)

      def al(r):
        return r if isinstance(r, int) else pl.multiple_of(r, 8)

      def w1job(r0, n):
        z = _ln(_ln(h_v[pl.ds(al(r0), n), :])).astype(bf16)
        g_v[pl.ds(al(r0 + 8), n), :] = _gelu(_dot(z, W(w1_v)))

      def shifted(r0, n):
        gw = g_v[pl.ds(al(r0), n + 16), :]
        return jnp.concatenate([gw[7:7 + n, 0:c4], gw[9:9 + n, c4:2 * c4],
                                gw[6:6 + n, 2 * c4:3 * c4], gw[10:10 + n, 3 * c4:]], axis=1).astype(bf16)

      def bbody(b, last):
        r = b * RB
        n = RB // 2
        slot = b % 2
        if not last:
          @pl.when(b >= 2)
          def _():
            out_cp(b - 2, slot).wait()
        else:
          out_cp(b - 2, slot).wait()
        hA = h_v[pl.ds(al(r), n), :]
        hB = h_v[pl.ds(al(r + n), n), :]
        x1A = _ln(hA) + _dot(shifted(r, n), W(w2_v))
        if not last:
          w1job(r + RB, n)
          tA = _gelu(_dot(_ln(x1A).astype(bf16), W(w3_v))).astype(bf16)
          x1B = _ln(hB) + _dot(shifted(r + n, n), W(w2_v))
          w1job(r + RB + n, n)
          oA = _dot(tA, W(w4_v))
          tB = _gelu(_dot(_ln(x1B).astype(bf16), W(w3_v))).astype(bf16)
        else:
          x1B = _ln(hB) + _dot(shifted(r + n, n), W(w2_v))
          tA = _gelu(_dot(_ln(x1A).astype(bf16), W(w3_v))).astype(bf16)
          tB = _gelu(_dot(_ln(x1B).astype(bf16), W(w3_v))).astype(bf16)
          oA = _dot(tA, W(w4_v))
        out_v[slot, pl.ds(0, n), :] = (hA + x1A + oA).astype(bf16)
        out_v[slot, pl.ds(n, n), :] = (hB + x1B + _dot(tB, W(w4_v))).astype(bf16)
        out_cp(b, slot).start()

      with jax.named_scope("b1first"):
        w1job(0, RB // 2)
        w1job(RB // 2, RB // 2)

      with jax.named_scope("bloop"):
        lax.fori_loop(0, NB - 1, lambda b, _: bbody(b, False), None)
      with jax.named_scope("blast"):
        bbody(NB - 1, True)
        out_cp(NB - 2, (NB - 2) % 2).wait()
        out_cp(NB - 1, (NB - 1) % 2).wait()
    else:
      if pdma:
        for c in b_cps:
          c.wait()
      out_v[0] = h_v[pl.ds(0, RB), :].astype(bf16)
      out_cp(0, 0).start()
      out_cp(0, 0).wait()

  scratch = [
      pltpu.VMEM((S, D), bf16),
      pltpu.VMEM((M, D), bf16),
      pltpu.VMEM((S, D), bf16),
      pltpu.VMEM((8, E), u32),
  ] + [pltpu.VMEM((HG, D // 2, E), u32)] * NU + [pltpu.VMEM((RG, HG * E), f32)] * NU + [
      pltpu.VMEM((N // 2, D), u32),
      pltpu.VMEM((S, D), f32),
      pltpu.VMEM((S + 16, D), f32),
      pltpu.VMEM((D // 2, D), u32), pltpu.VMEM((D // 2, D), u32),
      pltpu.VMEM((D // 2, F), u32), pltpu.VMEM((F // 2, D), u32),
      pltpu.VMEM((2, RB, D), bf16),
      pltpu.SemaphoreType.DMA((6,)),
      pltpu.SemaphoreType.DMA((NU + len(ramp),)),
      pltpu.SemaphoreType.DMA((8,)),
      pltpu.SemaphoreType.DMA((2,)),
  ]

  def fn(A_x, A_mem0, A_Wq, A_Wk, A_Wv, A_Wo, A_seg_len, B_x, B_w1, B_w2, B_w3, B_w4):
    del A_seg_len, B_x
    out = pl.pallas_call(
        kernel,
        in_specs=[pl.BlockSpec(memory_space=pltpu.SMEM)] + [pl.BlockSpec(memory_space=pl.ANY)] * 10,
        out_specs=pl.BlockSpec(memory_space=pl.ANY),
        out_shape=jax.ShapeDtypeStruct((S, D), bf16),
        scratch_shapes=scratch,
        compiler_params=pltpu.CompilerParams(vmem_limit_bytes=124 * 2**20),
        name=f"k2_{RB}_{phases}_{unroll}_{tag}",
    )(np.zeros((1,), np.int32), A_x.reshape(S, D), A_mem0.reshape(M, D),
      A_Wq.reshape(D // 2, 2 * H, E), A_Wk.reshape(D // 2, 2 * H, E), A_Wv.reshape(D // 2, 2 * H, E),
      A_Wo.reshape(N, D), B_w1, B_w2, B_w3, B_w4)
    return out.reshape(1, S, D)
  return fn


_KERNEL_FN = make_kernel()


@functools.partial(jax.jit, static_argnames=("A_seg_len",))
def pallas_sequential_preLN__memory_aug_recurrent_mem_tr__mixer_s_mlp__prompt_kernel(
    A_x, A_mem0, A_Wq, A_Wk, A_Wv, A_Wo, A_seg_len, B_x, B_w1, B_w2, B_w3, B_w4):
  assert int(A_seg_len) == SEG, "kernel is built for the reference's fixed segment length"
  assert A_x.shape == (1, S, D) and A_mem0.shape == (1, M, D) and A_Wq.shape == (D, H, E)
  assert B_w3.shape == (D, F)
  return _KERNEL_FN(A_x, A_mem0, A_Wq, A_Wk, A_Wv, A_Wo, A_seg_len, B_x, B_w1, B_w2, B_w3, B_w4)
```

```python
import functools

import jax
import jax.numpy as jnp
import numpy as np
from jax import lax
from jax.experimental import pallas as pl
from jax.experimental.pallas import tpu as pltpu

bf16 = jnp.bfloat16
f32 = jnp.float32
u32 = jnp.uint32

S, D, H, E, F = 2048, 1024, 32, 128, 3584
M, SEG = 8, 32
L = M + SEG
NSEG = S // SEG
N = H * E
R0 = 512
CH = 24
RG = 544
HG = 8
NG = H // HG
EPS = 1e-5
HP0 = SEG
GP0 = 2 * SEG


def _dot(a, b):
  return lax.dot_general(a, b, (((1,), (0,)), ((), ())), preferred_element_type=f32)


def _dot_nt(a, b):
  return lax.dot_general(a, b, (((1,), (1,)), ((), ())), preferred_element_type=f32)


def _ln(x):
  m = jnp.mean(x, axis=-1, keepdims=True)
  xc = x - m
  v = jnp.mean(xc * xc, axis=-1, keepdims=True)
  return xc * lax.rsqrt(v + EPS)


def _gelu(x):
  return 0.5 * x * (1.0 + jnp.tanh(0.7978845608028654 * (x + 0.044715 * (x * x * x))))


def _or_tree(ts):
  while len(ts) > 1:
    ts = [ts[i] | ts[i + 1] for i in range(0, len(ts) - 1, 2)] + ([ts[-1]] if len(ts) % 2 else [])
  return ts[0]


ORDERS = {
    'Y1': "q0 k0 v0 qk0 q1 k1 v1 pv0 qk1 q2 k2 v2 pv1 qk2 q3 k3 v3 pv2 qk3 wh0-4 wh4-8 wh8-12 wh12-16 pv3 wh16-20 wh20-24 wh24-28 wh28-32",
    'Y2': "q0 k0 v0 qk0 q1 k1 v1 pv0 qk1 q2 k2 v2 pv1 qk2 q3 k3 v3 pv2 qk3 wh0-8 wh8-16 pv3 wh16-20 wh20-24 wh24-28 wh28-32",
    'X2': "q0 k0 v0 qk0 q1 k1 v1 pv0 qk1 q2 k2 v2 pv1 qk2 q3 k3 v3 pv2 qk3 wo0-0 wo1-1 pv3 wo2-2 wo3-3",
    'J': "q0 k0 v0 qk0 q1 k1 v1 pv0 qk1 q2 k2 v2 pv1 qk2 q3 k3 v3 pv2 qk3 wo0-1 wo2-2 pv3 wo3-3",
    'L': "q0 k0 v0 qk0 q1 k1 v1 pv0 qk1 q2 k2 v2 pv1 qk2 q3 k3 v3 pv2 wo0-0 qk3 wo1-2 pv3 wo3-3",
    'F': "q0 k0 v0 qk0 q1 k1 pv0 v1 qk1 q2 k2 pv1 v2 qk2 q3 k3 pv2 qk3 v3 wo0-1 wo2-2 pv3 wo3-3",
}


def _parse(s):
  out = []
  for t in s.split():
    if t.startswith('wh'):
      a, b = t[2:].split('-')
      out.append(('wo', int(a), int(b)))
    elif t.startswith('wo'):
      a, b = t[2:].split('-')
      out.append(('wo', int(a) * HG, (int(b) + 1) * HG))
    elif t.startswith('qk'):
      out.append(('qk', int(t[2:])))
    elif t.startswith('pv'):
      out.append(('pv', int(t[2:])))
    else:
      out.append((t[0], int(t[1:])))
  return out


def make_kernel(order='Y1', RB=128, phases="PAB", unroll=4, bvar='halves2', tag='', ramp=((0, 0, 1), (0, 1, 2), (0, 2, 4), (1, 0, 2), (1, 2, 4)), nself=3, WSL=4, tdist=1, NSL=8, lnrows=16, pdma=False, usetie=True, noP=False, nodep=False, memfirst=False, noh=False, lnA=True, lnpos=('q', 1), lntie=('q', 2), WSL2={2: 6}, PD0=5, PDEP=3, x1at=8, tiemode='all', gtie=('k', 1), zpos=('v', 1), ztie=('q', 3)):
  scale = E ** -0.5
  NB = S // RB
  ops = _parse(ORDERS.get(order, order))
  NU = 3 * NG

  def kernel(z_smem, x_hbm, mem0_hbm, wq_hbm, wk_hbm, wv_hbm, wo_hbm, w1_hbm, w2_hbm, w3_hbm, w4_hbm,
             out_hbm, *scr):
    (x_v, mem_v, xln_v, z_v), scr = scr[:4], scr[4:]
    wpk, scr = scr[:NU], scr[NU:]
    ring, scr = scr[:NU], scr[NU:]
    (wo_pk, h_v, g_v, w1_v, w2_v, w3_v, w4_v, out_v,
     sem_x, sem_u, sem_w, sem_out) = scr
    whbm = [r.bitcast(u32) for r in (wq_hbm, wk_hbm, wv_hbm)]

    def unit_cps(u):
      m, g = divmod(u, NG)
      cps = []
      for par in range(2):
        for hpl in range(HG // 2):
          cps.append(pltpu.make_async_copy(
              whbm[m].at[:, par * (H // 2) + g * (HG // 2) + hpl, :],
              wpk[u].at[par * (HG // 2) + hpl], sem_u.at[u]))
      return cps

    x_cp1 = pltpu.make_async_copy(x_hbm.at[pl.ds(R0, S - R0)], x_v.at[pl.ds(R0, S - R0)], sem_x.at[4])
    mem_cp = pltpu.make_async_copy(mem0_hbm, mem_v, sem_x.at[5])
    NWO = 4
    wo_cps = [pltpu.make_async_copy(wo_hbm.bitcast(u32).at[pl.ds(i * (N // 2 // NWO), N // 2 // NWO)],
                                    wo_pk.at[pl.ds(i * (N // 2 // NWO), N // 2 // NWO)], sem_w.at[i])
              for i in range(NWO)]
    b_cps = [pltpu.make_async_copy(a.bitcast(u32), b, sem_w.at[NWO + i]) for i, (a, b) in enumerate(
        ((w1_hbm, w1_v), (w2_hbm, w2_v), (w3_hbm, w3_v), (w4_hbm, w4_v)))]

    off = len(ramp) - ramp[-1][0] - 1
    nsub = NU + off
    XW = nsub - 1 if lnA else off + 3
    extra = {(x1at if x1at is not None else off + 1): [x_cp1]}
    for j, c in enumerate(wo_cps):
      extra.setdefault(off + 3 + j, []).append(c)
    if "B" in phases or pdma:
      for j, c in enumerate(b_cps):
        extra.setdefault(off + 7 + j, []).append(c)
    lnplan = {}
    groups = list(range(R0, R0 + 32, lnrows)) if lnA else list(range(R0, S, lnrows))
    slots = [(i, sl) for i in range(XW, nsub) for sl in range(NSL - 1)]
    for j, r in enumerate(groups):
      lnplan.setdefault(slots[(j * len(slots)) // len(groups)], []).append(r)

    def fix_vals(ref, hpl, rows):
      a = ref[hpl, rows, :]
      c = ref[HG // 2 + hpl, rows, :]
      lo = (a & jnp.uint32(0xFFFF)) | (c << 16)
      hi = (a >> 16) | (c & jnp.uint32(0xFFFF0000))
      ref[hpl, rows, :] = lo
      ref[HG // 2 + hpl, rows, :] = hi
      return lo | hi

    def rhs(u):
      return pltpu.bitcast(jnp.concatenate(
          [wpk[u][(hl % 2) * (HG // 2) + hl // 2] for hl in range(HG)], axis=1), bf16)

    def ln_rows(r, n):
      y = _ln(x_v[pl.ds(r, n), :].astype(f32)).astype(bf16)
      xln_v[pl.ds(r, n), :] = y
      return y

    HP = HG // 2
    subs = list(ramp) + [(u, 0, HP) for u in range(ramp[-1][0] + 1, NU)]
    NSUB = len(subs)

    def sub_cps(i):
      u, a, b = subs[i]
      m, g = divmod(u, NG)
      return [pltpu.make_async_copy(
          whbm[m].at[:, par * (H // 2) + g * HP + hpl, :], wpk[u].at[par * HP + hpl], sem_u.at[i])
          for hpl in range(a, b) for par in range(2)]

    def start_all(cs):
      for c in cs:
        c.start()

    def wait_all(cs):
      for c in cs:
        c.wait()

    def wait_sub(i):
      u, a, b = subs[i]
      if (a, b) == (0, HP):
        pltpu.make_async_copy(wpk[u], wpk[u], sem_u.at[i]).wait()
      else:
        wait_all(sub_cps(i))

    def fix_chunk(i, r0, nrows):
      u, a, b = subs[i]
      acc = None
      for hpl in range(a, b):
        t = fix_vals(wpk[u], hpl, pl.ds(r0, nrows))
        qs = range(nrows // 8) if tiemode == 'all' else [nrows // 8 - 1]
        for q in qs:
          acc = t[8 * q:8 * q + 8] if acc is None else acc | t[8 * q:8 * q + 8]
      return acc

    def tie(lhs, dep):
      lu = pltpu.bitcast(lhs[0:16, 0:E], u32) | dep
      return jnp.concatenate(
          [jnp.concatenate([pltpu.bitcast(lu, bf16), lhs[0:16, E:]], axis=1), lhs[16:, :]], axis=0)

    zero = jnp.full((8, E), z_smem[0], jnp.int32).astype(u32)
    one = z_smem[0] + 1
    HU = whbm[0]
    NXC = 4
    XC = R0 // NXC

    def xc_cp(c):
      return pltpu.make_async_copy(x_hbm.at[pl.ds(c * XC, XC)], x_v.at[pl.ds(c * XC, XC)], sem_x.at[c])

    def in_block(fn, n=1):
      lax.fori_loop(0, one * n, lambda i, _: fn(i), None)

    def start_sub_dyn(i):
      u, a, b = subs[i]
      m, g = divmod(u, NG)

      def body(j):
        hpl = a + j // 2
        par = j % 2
        pltpu.make_async_copy(whbm[m].at[:, par * (H // 2) + g * HP + hpl, :],
                              wpk[u].at[par * HP + hpl], sem_u.at[i]).start()
      in_block(body, 2 * (b - a))

    in_block(lambda i: xc_cp(0).start())
    start_sub_dyn(0)
    in_block(lambda i: pltpu.make_async_copy(
        x_hbm.at[pl.ds(pl.multiple_of((i + 1) * XC, XC), XC)],
        x_v.at[pl.ds(pl.multiple_of((i + 1) * XC, XC), XC)], sem_x.at[i + 1]).start(), NXC - 1)
    for i in range(1, PD0):
      start_sub_dyn(i)
    mem_cp.start()

    started = [PD0]
    RS = R0 // NSL
    SPC = XC // RS

    def fix_all(i):
      for bb in range(8):
        fix_chunk(i, bb * 64, 64)

    for i, (u, a, b) in enumerate(subs):
      with jax.named_scope(f"unit{i:02d}"):
        c0, c1 = 2 * a * E, 2 * b * E
        deps = {}
        if i == 0:
          xc_cp(0).wait()
          ln_rows(0, XC)
          wait_all(sub_cps(0))
          fix_all(0)
        elif i < nself:
          wait_all(sub_cps(i))
          fix_all(i)
        for sl in range(NSL):
          if i == 0 and sl % SPC == 0 and sl // SPC + 1 < NXC:
            xc_cp(sl // SPC + 1).wait()
          if sl == WSL2.get(i, WSL) and i + 1 < NSUB:
            if i + 1 >= nself:
              wait_sub(i + 1)
            for j in range(started[0], min(i + PDEP + 1, NSUB)):
              start_all(sub_cps(j))
            started[0] = max(started[0], min(i + PDEP + 1, NSUB))
            for c in extra.get(i, ()):
              c.start()
          if sl == 0 and i == XW:
            x_cp1.wait()
          if noP:
            continue
          w = pltpu.bitcast(jnp.concatenate(
              [wpk[u][(hl % 2) * HP + hl // 2] for hl in range(2 * a, 2 * b)], axis=1), bf16)
          lhs = xln_v[pl.ds(sl * RS, RS), :]
          if sl in deps and usetie:
            lhs = tie(lhs, deps.pop(sl) & zero)
          ring[u][pl.ds(sl * RS, RS), c0:c1] = _dot(lhs, w)

          def add_dep(t, at):
            at = min(at, NSL - 1)
            if at > sl:
              deps[at] = t if at not in deps else deps[at] | t
          if i == 0 and sl % SPC == 0 and sl // SPC + 1 < NXC:
            ln_rows((sl // SPC + 1) * XC, XC)
          if nself <= i + 1 < NSUB and sl >= WSL2.get(i, WSL):
            ws = WSL2.get(i, WSL)
            nfs = max(NSL - 1 - ws, 1)
            k = sl - ws
            if k < nfs:
              lo, hi = (k * 64) // nfs * 8, ((k + 1) * 64) // nfs * 8
              if hi > lo:
                add_dep(fix_chunk(i + 1, lo, hi - lo), sl + tdist)
          for r in lnplan.get((i, sl), ()):
            y = ln_rows(r, lnrows)
            t = pltpu.bitcast(y[0:16, 0:E], u32)
            for q in range(1, lnrows // 16):
              t = t | pltpu.bitcast(y[16 * q:16 * q + 16, 0:E], u32)
            add_dep(t, sl + tdist)

    for c in wo_cps:
      c.wait()
    mem_cp.wait()
    if "B" in phases:
      b_cps[0].wait()
    h_v[pl.ds(0, HP0), :] = jnp.zeros((HP0, D), f32)
    z_v[...] = jnp.zeros((SEG, D), bf16)

    ri = lax.broadcasted_iota(jnp.int32, (L, L), 0)
    ci = lax.broadcasted_iota(jnp.int32, (L, L), 1)
    mask = (ri < M) | (ri >= ci)

    def step(s, carry):
      mem, wp, rpos = carry
      rc = pl.multiple_of(R0 + CH * s, 8)
      mem_in = mem
      if nodep:
        mem = mem_v[...].astype(f32)
      if memfirst:
        lhs = jnp.concatenate([mem.astype(bf16), xln_v[pl.ds(rc, CH), :]], axis=0)
      else:
        lhs = jnp.concatenate([xln_v[pl.ds(rc, CH), :], mem.astype(bf16)], axis=0)
      lnst = dict(dep=None, used=False)
      ties = {}
      if "B" in phases:
        gq = _gelu(_dot(z_v[...], pltpu.bitcast(w1_v[...], bf16)))
        g_v[pl.ds(pl.multiple_of(s * SEG, SEG), SEG), :] = gq
        d = None
        for i in range(SEG // 8):
          for q in range(D // E):
            t = pltpu.bitcast(gq[8 * i:8 * i + 8, q * E:(q + 1) * E], u32)
            d = t if d is None else d | t
        ties[gtie] = d
      t0 = M if memfirst else 0
      m0 = 0 if memfirst else CH
      wpos = [pl.multiple_of(wp, 8)]
      for i in range(CH // 8):
        t = wpos[-1] + 8
        wpos.append(pl.multiple_of(jnp.where(t >= RG, t - RG, t), 8))
      rpos = pl.multiple_of(rpos, SEG)
      rnext = jnp.where(rpos + SEG >= RG, 0, rpos + SEG)
      val = {}
      os_ = {}
      st = dict(acc=None)

      def proj(m, g):
        u = m * NG + g
        lh = lhs
        dd = ties.pop(('qkv'[m], g), None)
        if lnA and ('qkv'[m], g) == lntie:
          dd = lnst['dep'] if dd is None else dd | lnst['dep']
        if dd is not None:
          lh = tie(lhs, dd & zero)
        y = _dot(lh, rhs(u))
        if lnA and ('qkv'[m], g) == lnpos:
          rn = pl.multiple_of(jnp.minimum(rc + CH, S - CH), 8)
          yl = _ln(x_v[pl.ds(rn, CH), :].astype(f32)).astype(bf16)
          xln_v[pl.ds(rn, CH), :] = yl
          d = None
          for q in range(D // E):
            t = pltpu.bitcast(yl[0:16, q * E:(q + 1) * E], u32)
            d = t if d is None else d | t
          lnst['dep'] = d
        if "B" in phases and ('qkv'[m], g) == zpos:
          zz = _ln(_ln(h_v[pl.ds(pl.multiple_of(s * SEG, SEG), SEG), :])).astype(bf16)
          z_v[...] = zz
          d = None
          for i in range(SEG // 16):
            for q in range(D // E):
              t = pltpu.bitcast(zz[16 * i:16 * i + 16, q * E:(q + 1) * E], u32)
              d = t if d is None else d | t
          ties[ztie] = d if ztie not in ties else ties[ztie] | d
        for i in range(CH // 8):
          ring[u][pl.ds(wpos[i], 8), :] = y[t0 + 8 * i:t0 + 8 * (i + 1), :]
        val[(m, g)] = y[m0:m0 + M, :]

      def full(m, g):
        tok = ring[m * NG + g][pl.ds(rpos, SEG), :]
        return jnp.concatenate([val[(m, g)], tok], axis=0)

      def qk(g):
        q = full(0, g)
        k = full(1, g)
        for hh in range(HG):
          sl = slice(hh * E, (hh + 1) * E)
          sc = _dot_nt(q[:, sl], k[:, sl]) * scale
          sc = jnp.where(mask, sc, -1e9)
          mx = jnp.max(sc, axis=-1, keepdims=True)
          e = jnp.exp(sc - mx)
          l = jnp.sum(e, axis=-1, keepdims=True)
          r = pl.reciprocal(l, approx=True)
          r = r * (2.0 - l * r)
          val[('p', g * HG + hh)] = (e, r)

      def pv(g):
        v = full(2, g)
        for hh in range(HG):
          sl = slice(hh * E, (hh + 1) * E)
          e, r = val[('p', g * HG + hh)]
          os_[g * HG + hh] = _dot(e, v[:, sl]) * r

      def wo(h0, h1):
        o = jnp.concatenate([os_[h] for h in range(h0, h1)], axis=1)
        part = _dot(o, pltpu.bitcast(wo_pk[h0 * E // 2:h1 * E // 2, :], bf16))
        st['acc'] = part if st['acc'] is None else st['acc'] + part

      for op in ops:
        if op[0] == 'qk':
          qk(op[1])
        elif op[0] == 'pv':
          pv(op[1])
        elif op[0] == 'wo':
          wo(op[1], op[2])
        else:
          proj('qkv'.index(op[0]), op[1])
      acc = st['acc']
      r0 = pl.multiple_of(s * SEG, SEG)
      if noh:
        h_v[pl.ds(r0 + HP0, SEG), :] = acc[M:, :]
      else:
        h_v[pl.ds(r0 + HP0, SEG), :] = acc[M:, :] + x_v[pl.ds(r0, SEG), :].astype(f32)
      return acc[:M, :], wpos[CH // 8], rnext

    if "A" in phases:
      with jax.named_scope("steps"):
        lax.fori_loop(0, NSEG, step, (mem_v[...].astype(f32), jnp.int32(R0), jnp.int32(0)), unroll=unroll)
    else:
      for u in range(NU):
        h_v[pl.ds(HP0, RB), :] = x_v[pl.ds(0, RB), :].astype(f32) + ring[u][pl.ds(0, RB), :]

    def out_cp(b, slot):
      return pltpu.make_async_copy(out_v.at[slot], out_hbm.at[pl.ds(b * RB, RB)], sem_out.at[slot])

    if "B" in phases:
      for c in b_cps[1:]:
        c.wait()
      c4 = D // 4
      W = lambda r: pltpu.bitcast(r[...], bf16)

      def al(r):
        return r if isinstance(r, int) else pl.multiple_of(r, 8)

      W1 = pltpu.bitcast(w1_v[...], bf16)
      with jax.named_scope("gtail"):
        g_v[pl.ds(S, SEG), :] = _gelu(_dot(z_v[...], W1))
        zz = _ln(_ln(h_v[pl.ds(S, SEG), :])).astype(bf16)
        g_v[pl.ds(S + SEG, SEG), :] = _gelu(_dot(zz, W1))
      zero8 = jnp.zeros((8, D), f32)
      g_v[pl.ds(GP0 - 8, 8), :] = zero8
      g_v[pl.ds(GP0 + S, 8), :] = zero8

      def shifted(r0, n):
        gw = g_v[pl.ds(al(r0 + GP0 - 8), n + 16), :]
        return jnp.concatenate([gw[7:7 + n, 0:c4], gw[9:9 + n, c4:2 * c4],
                                gw[6:6 + n, 2 * c4:3 * c4], gw[10:10 + n, 3 * c4:]], axis=1).astype(bf16)

      def bbody(b, _):
        r = b * RB
        n = RB // 2
        slot = b % 2

        @pl.when(b >= 2)
        def _():
          out_cp(b - 2, slot).wait()
        hA = h_v[pl.ds(al(r + HP0), n), :]
        hB = h_v[pl.ds(al(r + HP0 + n), n), :]
        x1A = _ln(hA) + _dot(shifted(r, n), W(w2_v))
        x1B = _ln(hB) + _dot(shifted(r + n, n), W(w2_v))
        tA = _gelu(_dot(_ln(x1A).astype(bf16), W(w3_v))).astype(bf16)
        tB = _gelu(_dot(_ln(x1B).astype(bf16), W(w3_v))).astype(bf16)
        out_v[slot, pl.ds(0, n), :] = (hA + x1A + _dot(tA, W(w4_v))).astype(bf16)
        out_v[slot, pl.ds(n, n), :] = (hB + x1B + _dot(tB, W(w4_v))).astype(bf16)
        out_cp(b, slot).start()

      with jax.named_scope("bloop"):
        lax.fori_loop(0, NB, bbody, None)
      out_cp(NB - 2, (NB - 2) % 2).wait()
      out_cp(NB - 1, (NB - 1) % 2).wait()
    else:
      if pdma:
        for c in b_cps:
          c.wait()
      out_v[0] = h_v[pl.ds(HP0, RB), :].astype(bf16)
      out_cp(0, 0).start()
      out_cp(0, 0).wait()

  scratch = [
      pltpu.VMEM((S, D), bf16),
      pltpu.VMEM((M, D), bf16),
      pltpu.VMEM((S, D), bf16),
      pltpu.VMEM((SEG, D), bf16),
  ] + [pltpu.VMEM((HG, D // 2, E), u32)] * NU + [pltpu.VMEM((RG, HG * E), f32)] * NU + [
      pltpu.VMEM((N // 2, D), u32),
      pltpu.VMEM((HP0 + S, D), f32),
      pltpu.VMEM((GP0 + S + 8, D), f32),
      pltpu.VMEM((D // 2, D), u32), pltpu.VMEM((D // 2, D), u32),
      pltpu.VMEM((D // 2, F), u32), pltpu.VMEM((F // 2, D), u32),
      pltpu.VMEM((2, RB, D), bf16),
      pltpu.SemaphoreType.DMA((6,)),
      pltpu.SemaphoreType.DMA((NU + len(ramp),)),
      pltpu.SemaphoreType.DMA((8,)),
      pltpu.SemaphoreType.DMA((2,)),
  ]

  def fn(A_x, A_mem0, A_Wq, A_Wk, A_Wv, A_Wo, A_seg_len, B_x, B_w1, B_w2, B_w3, B_w4):
    del A_seg_len, B_x
    out = pl.pallas_call(
        kernel,
        in_specs=[pl.BlockSpec(memory_space=pltpu.SMEM)] + [pl.BlockSpec(memory_space=pl.ANY)] * 10,
        out_specs=pl.BlockSpec(memory_space=pl.ANY),
        out_shape=jax.ShapeDtypeStruct((S, D), bf16),
        scratch_shapes=scratch,
        compiler_params=pltpu.CompilerParams(vmem_limit_bytes=124 * 2**20),
        name=f"k2_{RB}_{phases}_{unroll}_{tag}",
    )(np.zeros((1,), np.int32), A_x.reshape(S, D), A_mem0.reshape(M, D),
      A_Wq.reshape(D // 2, 2 * H, E), A_Wk.reshape(D // 2, 2 * H, E), A_Wv.reshape(D // 2, 2 * H, E),
      A_Wo.reshape(N, D), B_w1, B_w2, B_w3, B_w4)
    return out.reshape(1, S, D)
  return fn


_KERNEL_FN = make_kernel()


@functools.partial(jax.jit, static_argnames=("A_seg_len",))
def pallas_sequential_preLN__memory_aug_recurrent_mem_tr__mixer_s_mlp__prompt_kernel(
    A_x, A_mem0, A_Wq, A_Wk, A_Wv, A_Wo, A_seg_len, B_x, B_w1, B_w2, B_w3, B_w4):
  assert int(A_seg_len) == SEG, "kernel is built for the reference's fixed segment length"
  assert A_x.shape == (1, S, D) and A_mem0.shape == (1, M, D) and A_Wq.shape == (D, H, E)
  assert B_w3.shape == (D, F)
  return _KERNEL_FN(A_x, A_mem0, A_Wq, A_Wk, A_Wv, A_Wo, A_seg_len, B_x, B_w1, B_w2, B_w3, B_w4)
```

```python
import functools

import jax
import jax.numpy as jnp
import numpy as np
from jax import lax
from jax.experimental import pallas as pl
from jax.experimental.pallas import tpu as pltpu

bf16 = jnp.bfloat16
f32 = jnp.float32
u32 = jnp.uint32

S, D, H, E, F = 2048, 1024, 32, 128, 3584
M, SEG = 8, 32
L = M + SEG
NSEG = S // SEG
N = H * E
EPS = 1e-5

R0 = 512
CH = 24
RG = 544
HG = 8
HP = HG // 2
NG = H // HG
NU = 3 * NG
HP0 = SEG
GP0 = 2 * SEG
RB = 128
NB = S // RB
NSL = 8
RS = R0 // NSL
NXC = 4
XC = R0 // NXC

RAMP = ((0, 0, 1), (0, 1, 2), (0, 2, 4), (1, 0, 2), (1, 2, 4))
SUBS = RAMP + tuple((u, 0, HP) for u in range(RAMP[-1][0] + 1, NU))
NSUB = len(SUBS)

ORDER = ("q0 k0 v0 qk0 q1 k1 v1 pv0 qk1 q2 k2 v2 pv1 qk2 q3 k3 v3 pv2 qk3 "
         "wo0-4 wo4-8 wo8-12 wo12-16 pv3 wo16-20 wo20-24 wo24-28 wo28-32")


def _dot(a, b):
  return lax.dot_general(a, b, (((1,), (0,)), ((), ())), preferred_element_type=f32)


def _dot_nt(a, b):
  return lax.dot_general(a, b, (((1,), (1,)), ((), ())), preferred_element_type=f32)


def _ln(x):
  m = jnp.mean(x, axis=-1, keepdims=True)
  xc = x - m
  v = jnp.mean(xc * xc, axis=-1, keepdims=True)
  return xc * lax.rsqrt(v + EPS)


def _gelu(x):
  return 0.5 * x * (1.0 + jnp.tanh(0.7978845608028654 * (x + 0.044715 * (x * x * x))))


def _as_bf16(ref_or_val):
  return pltpu.bitcast(ref_or_val, bf16)


def _or_chain(vals):
  acc = None
  for t in vals:
    acc = t if acc is None else acc | t
  return acc


def _kernel(z_smem, x_hbm, mem0_hbm, wq_hbm, wk_hbm, wv_hbm, wo_hbm,
            w1_hbm, w2_hbm, w3_hbm, w4_hbm, out_hbm, *scr):
  (x_v, mem_v, xln_v, z_v), scr = scr[:4], scr[4:]
  wpk, scr = scr[:NU], scr[NU:]
  ring, scr = scr[:NU], scr[NU:]
  (wo_v, h_v, g_v, w1_v, w2_v, w3_v, w4_v, out_v, sem_x, sem_u, sem_w, sem_out) = scr

  whbm = [r.bitcast(u32) for r in (wq_hbm, wk_hbm, wv_hbm)]

  def w_copy(i, hpl, par):
    u = SUBS[i][0]
    m, g = divmod(u, NG)
    return pltpu.make_async_copy(
        whbm[m].at[:, par * (H // 2) + g * HP + hpl, :], wpk[u].at[par * HP + hpl], sem_u.at[i])

  def sub_copies(i):
    _, a, b = SUBS[i]
    return [w_copy(i, hpl, par) for hpl in range(a, b) for par in range(2)]

  def start_sub(i):
    for c in sub_copies(i):
      c.start()

  def start_sub_ordered(i):
    _, a, b = SUBS[i]
    lax.fori_loop(0, 2 * (b - a), lambda j, _: w_copy(i, a + j // 2, j % 2).start(), None)

  def wait_sub(i):
    u, a, b = SUBS[i]
    if (a, b) == (0, HP):
      pltpu.make_async_copy(wpk[u], wpk[u], sem_u.at[i]).wait()
    else:
      for c in sub_copies(i):
        c.wait()

  def x_rows_copy(r, n, sem):
    return pltpu.make_async_copy(x_hbm.at[pl.ds(r, n)], x_v.at[pl.ds(r, n)], sem)

  def x_half(j):
    return x_rows_copy(pl.multiple_of(j * (XC // 2), XC // 2), XC // 2, sem_x.at[0])

  def x_chunk(c):
    return x_rows_copy(pl.multiple_of(c * XC, XC), XC, sem_x.at[c])

  x_rest = x_rows_copy(R0, S - R0, sem_x.at[NXC])
  mem_cp = pltpu.make_async_copy(mem0_hbm, mem_v, sem_x.at[NXC + 1])
  NWO = 4
  wo_rows = N // 2 // NWO
  wo_cps = [pltpu.make_async_copy(wo_hbm.bitcast(u32).at[pl.ds(i * wo_rows, wo_rows)],
                                  wo_v.at[pl.ds(i * wo_rows, wo_rows)], sem_w.at[i])
            for i in range(NWO)]
  b_cps = [pltpu.make_async_copy(a.bitcast(u32), b, sem_w.at[NWO + i]) for i, (a, b) in enumerate(
      ((w1_hbm, w1_v), (w2_hbm, w2_v), (w3_hbm, w3_v), (w4_hbm, w4_v)))]
  extra = {8: [x_rest]}
  for j, c in enumerate(wo_cps):
    extra.setdefault(6 + j, []).append(c)
  for j, c in enumerate(b_cps):
    extra.setdefault(10 + j, []).append(c)

  def fix_rows(i, r0, nrows):
    u, a, b = SUBS[i]
    rows = pl.ds(r0, nrows)
    acc = None
    for hpl in range(a, b):
      even = wpk[u][hpl, rows, :]
      odd = wpk[u][HP + hpl, rows, :]
      lo = (even & jnp.uint32(0xFFFF)) | (odd << 16)
      hi = (even >> 16) | (odd & jnp.uint32(0xFFFF0000))
      wpk[u][hpl, rows, :] = lo
      wpk[u][HP + hpl, rows, :] = hi
      t = lo | hi
      for q in range(nrows // 8):
        acc = t[8 * q:8 * q + 8] if acc is None else acc | t[8 * q:8 * q + 8]
    return acc

  def fix_all(i):
    for b in range(8):
      fix_rows(i, b * 64, 64)

  def w_block(u, h0=0, h1=HG):
    return _as_bf16(jnp.concatenate(
        [wpk[u][(hl % 2) * HP + hl // 2] for hl in range(h0, h1)], axis=1))

  def ln_rows(r, n):
    y = _ln(x_v[pl.ds(r, n), :].astype(f32)).astype(bf16)
    xln_v[pl.ds(r, n), :] = y
    return y

  zero = jnp.full((8, E), z_smem[0], jnp.int32).astype(u32)

  def tie(lhs, dep):
    lu = pltpu.bitcast(lhs[0:16, 0:E], u32) | (dep & zero)
    top = jnp.concatenate([_as_bf16(lu), lhs[0:16, E:]], axis=1)
    return jnp.concatenate([top, lhs[16:, :]], axis=0)

  lax.fori_loop(0, 2, lambda j, _: x_half(j).start(), None)
  start_sub_ordered(0)
  lax.fori_loop(1, NXC, lambda c, _: x_chunk(c).start(), None)
  for i in range(1, len(RAMP)):
    start_sub_ordered(i)
  mem_cp.start()

  started = len(RAMP)
  spc = XC // RS
  for i, (u, a, b) in enumerate(SUBS):
    wsl = 6 if i == 2 else 4
    deps = {}
    if i == 0:
      x_half(0).wait()
      x_half(1).wait()
      ln_rows(0, XC)
    if i < 3:
      wait_sub(i)
      fix_all(i)
    for sl in range(NSL):
      if i == 0 and sl % spc == 0 and sl // spc + 1 < NXC:
        x_chunk(sl // spc + 1).wait()
      if sl == wsl and i + 1 < NSUB:
        if i + 1 >= 3:
          wait_sub(i + 1)
        for j in range(started, min(i + 4, NSUB)):
          start_sub(j)
        started = max(started, min(i + 4, NSUB))
        for c in extra.get(i, ()):
          c.start()
      if sl == 0 and i == NSUB - 1:
        x_rest.wait()
      lhs = xln_v[pl.ds(sl * RS, RS), :]
      if sl in deps:
        lhs = tie(lhs, deps.pop(sl))
      ring[u][pl.ds(sl * RS, RS), 2 * a * E:2 * b * E] = _dot(lhs, w_block(u, 2 * a, 2 * b))

      dep = []
      if i == 0 and sl % spc == 0 and sl // spc + 1 < NXC:
        ln_rows((sl // spc + 1) * XC, XC)
      if 3 <= i + 1 < NSUB and wsl <= sl < NSL - 1:
        nfs = NSL - 1 - wsl
        k = sl - wsl
        lo, hi = (k * 64) // nfs * 8, ((k + 1) * 64) // nfs * 8
        dep.append(fix_rows(i + 1, lo, hi - lo))
      if i == NSUB - 1 and sl in (0, 3):
        y = ln_rows(R0 + (16 if sl else 0), 16)
        dep.append(pltpu.bitcast(y[:, 0:E], u32))
      if dep and sl + 1 < NSL:
        deps[sl + 1] = _or_chain(dep)

  for c in wo_cps:
    c.wait()
  mem_cp.wait()
  b_cps[0].wait()
  h_v[pl.ds(0, HP0), :] = jnp.zeros((HP0, D), f32)
  z_v[...] = jnp.zeros((SEG, D), bf16)

  ri = lax.broadcasted_iota(jnp.int32, (L, L), 0)
  ci = lax.broadcasted_iota(jnp.int32, (L, L), 1)
  mask = (ri < M) | (ri >= ci)
  scale = E ** -0.5

  def step(s, carry):
    mem, wp, rpos = carry
    rc = pl.multiple_of(R0 + CH * s, 8)
    lhs = jnp.concatenate([xln_v[pl.ds(rc, CH), :], mem.astype(bf16)], axis=0)
    wpos = [pl.multiple_of(wp, 8)]
    for _ in range(CH // 8):
      t = wpos[-1] + 8
      wpos.append(pl.multiple_of(jnp.where(t >= RG, t - RG, t), 8))
    rpos = pl.multiple_of(rpos, SEG)
    rnext = jnp.where(rpos + SEG >= RG, 0, rpos + SEG)
    r0 = pl.multiple_of(s * SEG, SEG)

    gq = _gelu(_dot(z_v[...], _as_bf16(w1_v[...])))
    g_v[pl.ds(r0, SEG), :] = gq
    ties = {"k1": _or_chain(pltpu.bitcast(gq[8 * i:8 * i + 8, q * E:(q + 1) * E], u32)
                            for i in range(SEG // 8) for q in range(D // E))}

    memrows = {}
    probs = {}
    heads = {}
    acc = None

    def full(m, g, hh):
      sl = slice(hh * E, (hh + 1) * E)
      return jnp.concatenate([memrows[m, g][:, sl], ring[m * NG + g][pl.ds(rpos, SEG), sl]], axis=0)

    for op in ORDER.split():
      if op.startswith("qk"):
        g = int(op[2])
        for hh in range(HG):
          sc = _dot_nt(full(0, g, hh), full(1, g, hh)) * scale
          sc = jnp.where(mask, sc, -1e9)
          e = jnp.exp(sc - jnp.max(sc, axis=-1, keepdims=True))
          l = jnp.sum(e, axis=-1, keepdims=True)
          r = pl.reciprocal(l, approx=True)
          probs[g * HG + hh] = (e, r * (2.0 - l * r))
      elif op.startswith("pv"):
        g = int(op[2])
        for hh in range(HG):
          e, r = probs[g * HG + hh]
          heads[g * HG + hh] = _dot(e, full(2, g, hh)) * r
      elif op.startswith("wo"):
        h0, h1 = (int(t) for t in op[2:].split("-"))
        o = jnp.concatenate([heads[h] for h in range(h0, h1)], axis=1)
        part = _dot(o, _as_bf16(wo_v[h0 * E // 2:h1 * E // 2, :]))
        acc = part if acc is None else acc + part
      else:
        m, g = "qkv".index(op[0]), int(op[1])
        u = m * NG + g
        y = _dot(tie(lhs, ties.pop(op)) if op in ties else lhs, w_block(u))
        for i in range(CH // 8):
          ring[u][pl.ds(wpos[i], 8), :] = y[8 * i:8 * (i + 1), :]
        memrows[m, g] = y[CH:, :]
        if op == "q1":
          rn = pl.multiple_of(jnp.minimum(rc + CH, S - CH), 8)
          yl = ln_rows(rn, CH)
          ties["q2"] = _or_chain(pltpu.bitcast(yl[0:16, q * E:(q + 1) * E], u32)
                                 for q in range(D // E))
        if op == "v1":
          zz = _ln(_ln(h_v[pl.ds(r0, SEG), :])).astype(bf16)
          z_v[...] = zz
          ties["q3"] = _or_chain(pltpu.bitcast(zz[16 * i:16 * i + 16, q * E:(q + 1) * E], u32)
                                 for i in range(SEG // 16) for q in range(D // E))
    h_v[pl.ds(r0 + HP0, SEG), :] = acc[M:, :] + x_v[pl.ds(r0, SEG), :].astype(f32)
    return acc[:M, :], wpos[CH // 8], rnext

  lax.fori_loop(0, NSEG, step, (mem_v[...].astype(f32), jnp.int32(R0), jnp.int32(0)), unroll=4)

  for c in b_cps[1:]:
    c.wait()
  w1 = _as_bf16(w1_v[...])
  g_v[pl.ds(S, SEG), :] = _gelu(_dot(z_v[...], w1))
  zz = _ln(_ln(h_v[pl.ds(S, SEG), :])).astype(bf16)
  g_v[pl.ds(S + SEG, SEG), :] = _gelu(_dot(zz, w1))
  g_v[pl.ds(GP0 - 8, 8), :] = jnp.zeros((8, D), f32)
  g_v[pl.ds(GP0 + S, 8), :] = jnp.zeros((8, D), f32)
  c4 = D // 4

  def out_cp(b, slot):
    return pltpu.make_async_copy(out_v.at[slot], out_hbm.at[pl.ds(b * RB, RB)], sem_out.at[slot])

  def shifted(r, n):
    gw = g_v[pl.ds(pl.multiple_of(r + GP0 - 8, 8), n + 16), :]
    return jnp.concatenate([gw[7:7 + n, 0:c4], gw[9:9 + n, c4:2 * c4],
                            gw[6:6 + n, 2 * c4:3 * c4], gw[10:10 + n, 3 * c4:]],
                           axis=1).astype(bf16)

  def block(b, _):
    r = b * RB
    n = RB // 2
    slot = b % 2

    @pl.when(b >= 2)
    def _():
      out_cp(b - 2, slot).wait()

    ha = h_v[pl.ds(pl.multiple_of(r + HP0, 8), n), :]
    hb = h_v[pl.ds(pl.multiple_of(r + HP0 + n, 8), n), :]
    xa = _ln(ha) + _dot(shifted(r, n), _as_bf16(w2_v[...]))
    xb = _ln(hb) + _dot(shifted(r + n, n), _as_bf16(w2_v[...]))
    ta = _gelu(_dot(_ln(xa).astype(bf16), _as_bf16(w3_v[...]))).astype(bf16)
    tb = _gelu(_dot(_ln(xb).astype(bf16), _as_bf16(w3_v[...]))).astype(bf16)
    out_v[slot, pl.ds(0, n), :] = (ha + xa + _dot(ta, _as_bf16(w4_v[...]))).astype(bf16)
    out_v[slot, pl.ds(n, n), :] = (hb + xb + _dot(tb, _as_bf16(w4_v[...]))).astype(bf16)
    out_cp(b, slot).start()

  lax.fori_loop(0, NB, block, None)
  out_cp(NB - 2, (NB - 2) % 2).wait()
  out_cp(NB - 1, (NB - 1) % 2).wait()


def _scratch_shapes():
  return [
      pltpu.VMEM((S, D), bf16),
      pltpu.VMEM((M, D), bf16),
      pltpu.VMEM((S, D), bf16),
      pltpu.VMEM((SEG, D), bf16),
  ] + [pltpu.VMEM((HG, D // 2, E), u32)] * NU + [pltpu.VMEM((RG, HG * E), f32)] * NU + [
      pltpu.VMEM((N // 2, D), u32),
      pltpu.VMEM((HP0 + S, D), f32),
      pltpu.VMEM((GP0 + S + 8, D), f32),
      pltpu.VMEM((D // 2, D), u32), pltpu.VMEM((D // 2, D), u32),
      pltpu.VMEM((D // 2, F), u32), pltpu.VMEM((F // 2, D), u32),
      pltpu.VMEM((2, RB, D), bf16),
      pltpu.SemaphoreType.DMA((NXC + 2,)),
      pltpu.SemaphoreType.DMA((NSUB,)),
      pltpu.SemaphoreType.DMA((8,)),
      pltpu.SemaphoreType.DMA((2,)),
  ]


@functools.partial(jax.jit, static_argnames=("A_seg_len",))
def pallas_sequential_preLN__memory_aug_recurrent_mem_tr__mixer_s_mlp__prompt_kernel(
    A_x, A_mem0, A_Wq, A_Wk, A_Wv, A_Wo, A_seg_len, B_x, B_w1, B_w2, B_w3, B_w4):
  del B_x
  assert int(A_seg_len) == SEG, "built for the reference's fixed segment length"
  assert A_x.shape == (1, S, D) and A_mem0.shape == (1, M, D)
  assert A_Wq.shape == A_Wk.shape == A_Wv.shape == (D, H, E) and A_Wo.shape == (H, E, D)
  assert B_w1.shape == B_w2.shape == (D, D) and B_w3.shape == (D, F) and B_w4.shape == (F, D)
  out = pl.pallas_call(
      _kernel,
      in_specs=[pl.BlockSpec(memory_space=pltpu.SMEM)] + [pl.BlockSpec(memory_space=pl.ANY)] * 10,
      out_specs=pl.BlockSpec(memory_space=pl.ANY),
      out_shape=jax.ShapeDtypeStruct((S, D), bf16),
      scratch_shapes=_scratch_shapes(),
      compiler_params=pltpu.CompilerParams(vmem_limit_bytes=124 * 2**20),
      name="rmt_mixer_fused",
  )(np.zeros((1,), np.int32), A_x.reshape(S, D), A_mem0.reshape(M, D),
    A_Wq.reshape(D // 2, 2 * H, E), A_Wk.reshape(D // 2, 2 * H, E), A_Wv.reshape(D // 2, 2 * H, E),
    A_Wo.reshape(N, D), B_w1, B_w2, B_w3, B_w4)
  return out.reshape(1, S, D)
```
